```python
import os as _os
_os.environ.setdefault("JAX_PLATFORMS", "cpu")
import jax
import jax.numpy as jnp

def _softmax(x, axis=-1):
    return jax.nn.softmax(x, axis=axis)
def _gelu(x):
    return jax.nn.gelu(x, approximate=True)
def _silu(x):
    return jax.nn.silu(x)
def _sigmoid(x):
    return jax.nn.sigmoid(x)
def _layernorm(x, axis=-1, eps=1e-5):
    m = jnp.mean(x, axis=axis, keepdims=True)
    v = jnp.var(x, axis=axis, keepdims=True)
    return (x - m) / jnp.sqrt(v + eps)
def _scatter_add(tgt, idx, src, axis=0):
    return tgt.at[idx].add(src)
def _segment_sum(src, seg, n):
    return jax.ops.segment_sum(src, seg, n)
class _Rng:
    def __init__(self, key):
        self._k = key
    def _next(self):
        self._k, sub = jax.random.split(self._k)
        return sub
    def normal(self, shape):
        return jax.random.normal(self._next(), shape, dtype=jnp.bfloat16)
    def randint(self, lo, hi, shape):
        return jax.random.randint(self._next(), shape, lo, hi, dtype=jnp.int32)
    def uniform(self, shape, lo=0.0, hi=1.0):
        return jax.random.uniform(self._next(), shape, jnp.bfloat16, lo, hi)
    def permutation(self, n):
        return jax.random.permutation(self._next(), n)


kernel_name = 'parallel_sum__softmax_full_mha__moe_arch_mod__prompt'

def setup_inputs():
    _rng = _Rng(jax.random.key(int.from_bytes(__import__("os").urandom(4), "little")))
    _w = (lambda a: (lambda t: t.astype(jnp.bfloat16) if jnp.issubdtype(t.dtype, jnp.floating) else t)(jnp.asarray(a)))
    def _A_setup():
        B, S, D = 1, 2048, 512
        return {
            "x": _w((lambda *s: _rng.normal(s) * 0.05)(B, S, D)),
            "wqkv": _w((lambda *s: _rng.normal(s) * 0.1)(D, 3 * D)),
            "wo": _w((lambda *s: _rng.normal(s) * 0.05)(D, D)),
        }
    _A_in = _A_setup()

    def _B_setup():
        B, S, D, F, C = 1, 2048, 512, 1792, 1
        return {
            "x": _w((lambda *s: _rng.normal(s) * 0.05)(B, S, D)),
            "w_r": _w((lambda *s: _rng.normal(s) * 1.6)(D)),
            "w_gate": _w((lambda *s: _rng.normal(s) * 0.1)(D, F)),
            "w_up": _w((lambda *s: _rng.normal(s) * 0.1)(D, F)),
            "w_down": _w((lambda *s: _rng.normal(s) * 0.1)(F, D)),
        }
    _B_in = _B_setup()

    return {
        "A_x": _A_in["x"],
        "A_wqkv": _A_in["wqkv"],
        "A_wo": _A_in["wo"],
        "B_x": _B_in["x"],
        "B_w_r": _B_in["w_r"],
        "B_w_gate": _B_in["w_gate"],
        "B_w_up": _B_in["w_up"],
        "B_w_down": _B_in["w_down"],
    }

def reference(A_x, A_wqkv, A_wo, B_x, B_w_r, B_w_gate, B_w_up, B_w_down):
    def _A_ref(x, wqkv, wo):
        B, S, D = x.shape
        H = 32; Dh = D // H
        qkv = (lambda x, *d: x.transpose(*d))((x @ wqkv).reshape(B, S, 3, H, Dh), 2, 0, 3, 1, 4)
        q, k, v = qkv[0], qkv[1], qkv[2]
        scale = Dh ** -0.5
        scores = jnp.einsum("bhqd,bhkd->bhqk", q, k) * scale
        p = _softmax(scores, axis=-1)
        o = jnp.einsum("bhqk,bhkd->bhqd", p, v)
        return (lambda x, *d: x.transpose(*d))(o, 0, 2, 1, 3).reshape(B, S, D) @ wo

    def _B_ref(x, w_r, w_gate, w_up, w_down):
        B, S, D = x.shape
        C = 1
        r = x @ w_r
        idx = jnp.argsort(-r, axis=-1)[:, :C]
        idx_e = jnp.repeat(idx.reshape(B, C, 1), D, axis=2)
        x_sel = jnp.take_along_axis(x, idx_e, axis=1)
        g = _silu(x_sel @ w_gate)
        u = x_sel @ w_up
        y = (g * u) @ w_down
        r_sel = _sigmoid(jnp.take_along_axis(r, idx, axis=1))
        y = y * r_sel.reshape(B, C, 1)
        b_off = (jnp.arange(B) * S).reshape(B, 1)
        flat_idx = (idx + b_off).reshape(B * C)
        zero = (x * 0.0).reshape(B * S, D)
        upd = _scatter_add(zero, flat_idx, y.reshape(B * C, D), axis=0)
        return x + upd.reshape(B, S, D)

    x = A_x
    xn = _layernorm(x, axis=-1)
    return x + _A_ref(xn, A_wqkv, A_wo) + _B_ref(xn, B_w_r, B_w_gate, B_w_up, B_w_down)
```

```python
import functools
import jax
import jax.numpy as jnp
import jax.experimental.pallas as pl
import jax.experimental.pallas.tpu as pltpu

S, D, H, DH, F = 2048, 512, 32, 16, 1792
G = 128 // DH
NG = H // G
LOG2E = 1.4426950408889634
bf16 = jnp.bfloat16
f32 = jnp.float32


def _rb(x):
    return x.astype(bf16).astype(f32)


def make_kernel(TQ, order, NC, UB, serial):
    NQ = S // TQ
    NU = NQ * H
    KC = S // NC

    def kernel(x_ref, wqkv_ref, wo_hbm, wr_ref, wg_hbm, wu_hbm, wd_hbm, o_ref,
               xn_ref, k_ref, qt_ref, vt_ref, ot_ref, y_ref, idx_ref, xsel_ref, rs_ref,
               wo_ref, wg_ref, wu_ref, wd_ref, sems, *sm):
        s_refs = sm[:2 * UB]
        m_refs = sm[2 * UB:]
        copies = [pltpu.make_async_copy(src, dst, sems.at[i]) for i, (src, dst) in enumerate(
            ((wo_hbm, wo_ref), (wg_hbm, wg_ref), (wu_hbm, wu_ref), (wd_hbm, wd_ref)))]
        qi = pl.program_id(0)
        row = jax.lax.broadcasted_iota(jnp.int32, (128, TQ), 0) // DH

        def qmask(u):
            u = jnp.minimum(u, NU - 1)
            qq = u // H
            h = u % H
            g = h // G
            hh = h % G
            qg = qt_ref[qq, pl.ds(pl.multiple_of(g * 128, 128), 128), :]
            return g, jnp.where(row == hh, qg, jnp.zeros_like(qg))

        def qk(u, s_ref, m_ref):
            g, qm = qmask(u)
            s = jnp.dot(k_ref[g], qm, preferred_element_type=f32)
            s_ref[...] = s
            m_ref[...] = jnp.broadcast_to(jnp.max(s, axis=0, keepdims=True), (8, TQ))

        @pl.when(qi == 0)
        def _prologue():
            for cp in copies:
                cp.start()
            xf = x_ref[...].astype(f32)
            mean = jnp.mean(xf, axis=-1, keepdims=True)
            cen = xf - mean
            var = jnp.mean(cen * cen, axis=-1, keepdims=True)
            m_b = _rb(mean)
            v_b = _rb(var)
            d_b = _rb(xf - m_b)
            den = _rb(jnp.sqrt(_rb(v_b + 1e-5)))
            xn = (d_b / den).astype(bf16)
            xn_ref[...] = xn
            wq = wqkv_ref[:, 0:D]
            wk = wqkv_ref[:, D:2 * D]
            wv = wqkv_ref[:, 2 * D:3 * D]
            k = jnp.dot(xn, wk, preferred_element_type=f32).astype(bf16)
            for g in range(NG):
                k_ref[g] = k[:, g * 128:(g + 1) * 128]
            qt = jax.lax.dot_general(wq, xn, (((0,), (1,)), ((), ())), preferred_element_type=f32)
            qt = (_rb(qt) * (DH ** -0.5 * LOG2E)).astype(bf16)
            for i in range(NQ):
                qt_ref[i] = qt[:, i * TQ:(i + 1) * TQ]
            vt_ref[...] = jax.lax.dot_general(wv, xn, (((0,), (1,)), ((), ())), preferred_element_type=f32).astype(bf16)
            wr = jnp.broadcast_to(wr_ref[...], (8, D))
            r = jax.lax.dot_general(wr, xn, (((1,), (1,)), ((), ())), preferred_element_type=f32)
            r = _rb(r)
            rmax = jnp.max(r, axis=-1, keepdims=True)
            lane = jax.lax.broadcasted_iota(jnp.int32, (8, S), 1)
            idx = jnp.min(jnp.where(r == rmax, lane, S), axis=-1, keepdims=True)
            onehot = (lane == idx).astype(bf16)
            x_sel = jnp.dot(onehot, xn, preferred_element_type=f32).astype(bf16)
            xsel_ref[...] = x_sel
            rs_ref[...] = jnp.broadcast_to(_rb(jax.nn.sigmoid(rmax)), (8, 128))
            idx_ref[...] = jnp.broadcast_to(idx, (8, 128))
            for t in range(UB):
                qk(t, s_refs[t], m_refs[t])

        def unit(u, sa, ma, sb, mb, do_qk=True):
            if do_qk:
                g, qm = qmask(u + UB)
            mb_v = mb[0:1, :]
            h = u % H
            hrow = pl.multiple_of(h * DH, DH)
            macc = None
            oacc = None
            lacc = None
            for c in range(NC):
                ks = slice(c * KC, (c + 1) * KC)
                for ch in order:
                    if ch == 'q':
                        if not do_qk:
                            continue
                        s = jnp.dot(k_ref[g, ks, :], qm, preferred_element_type=f32)
                        sa[ks, :] = s
                        mc = jnp.max(s.reshape(KC // 8, 8, TQ), axis=0)
                        macc = mc if macc is None else jnp.maximum(macc, mc)
                    else:
                        pf = jnp.exp2(sb[ks, :] - mb_v)
                        if serial:
                            for i in range(KC // 8):
                                lc = pf[8 * i:8 * i + 8, :]
                                lacc = lc if lacc is None else lacc + lc
                        else:
                            lc = jnp.sum(pf.reshape(KC // 8, 8, TQ), axis=0)
                            lacc = lc if lacc is None else lacc + lc
                        p = pf.astype(bf16)
                        o = jnp.dot(vt_ref[pl.ds(hrow, DH), ks], p, preferred_element_type=f32)
                        oacc = o if oacc is None else oacc + o
            if do_qk:
                ma[...] = jnp.broadcast_to(jnp.max(macc, axis=0, keepdims=True), (8, TQ))
            o = oacc / jnp.sum(lacc, axis=0, keepdims=True)
            ot_ref[pl.ds(hrow, DH), :] = o.astype(bf16)

        def body(j, carry):
            u = qi * H + UB * j
            last = u + UB >= NU
            for par, cond, do_qk in ((0, j % 2 == 0, True),
                                     (1, jnp.logical_and(j % 2 == 1, jnp.logical_not(last)), True),
                                     (1, last, False)):
                @pl.when(cond)
                def _():
                    for t in range(UB):
                        rd = par * UB + t
                        wr = (1 - par) * UB + t
                        unit(u + t, s_refs[wr], m_refs[wr], s_refs[rd], m_refs[rd], do_qk)
            return carry

        jax.lax.fori_loop(0, H // UB, body, 0)

        @pl.when(qi == 0)
        def _ffn():
            for cp in copies:
                cp.wait()
            x_sel = xsel_ref[...]
            gg = _rb(jnp.dot(x_sel, wg_ref[...], preferred_element_type=f32))
            gg = _rb(gg * jax.nn.sigmoid(gg))
            uu = _rb(jnp.dot(x_sel, wu_ref[...], preferred_element_type=f32))
            gu = (gg * uu).astype(bf16)
            y = _rb(jnp.dot(gu, wd_ref[...], preferred_element_type=f32))
            y_ref[...] = _rb(y * rs_ref[:, 0:1])

        q0 = pl.multiple_of(qi * TQ, TQ)
        a = jax.lax.dot_general(ot_ref[...], wo_ref[...], (((0,), (0,)), ((), ())), preferred_element_type=f32)
        xt = x_ref[pl.ds(q0, TQ), :].astype(f32)
        xnt = xn_ref[pl.ds(q0, TQ), :].astype(f32)
        rows = jax.lax.broadcasted_iota(jnp.int32, (TQ, D), 0) + q0
        idx = idx_ref[0:1, 0:1]
        upd = jnp.where(rows == idx, y_ref[0:1, :], 0.0)
        o_ref[...] = (_rb(xt + _rb(a)) + _rb(xnt + upd)).astype(o_ref.dtype)

    return kernel, NQ


@jax.jit
def pallas_parallel_sum__softmax_full_mha__moe_arch_mod__prompt_kernel(
    A_x: jax.Array,
    A_wqkv: jax.Array,
    A_wo: jax.Array,
    B_x: jax.Array,
    B_w_r: jax.Array,
    B_w_gate: jax.Array,
    B_w_up: jax.Array,
    B_w_down: jax.Array,
):
    TQ, order, NC, UB, serial = 512, "qp", 16, 4, True
    x = A_x.reshape(S, D)
    wr = B_w_r.reshape(1, D)
    kernel, NQ = make_kernel(TQ, order, NC, UB, serial)
    full = lambda shp: pl.BlockSpec(shp, lambda i: (0,) * len(shp))
    anyspec = pl.BlockSpec(memory_space=pl.ANY)
    out = pl.pallas_call(
        kernel,
        grid=(NQ,),
        in_specs=[full((S, D)), full((D, 3 * D)), anyspec, full((1, D)),
                  anyspec, anyspec, anyspec],
        out_specs=pl.BlockSpec((TQ, D), lambda i: (i, 0)),
        out_shape=jax.ShapeDtypeStruct((S, D), bf16),
        scratch_shapes=[
            pltpu.VMEM((S, D), bf16),
            pltpu.VMEM((NG, S, 128), bf16),
            pltpu.VMEM((NQ, D, TQ), bf16),
            pltpu.VMEM((D, S), bf16),
            pltpu.VMEM((D, TQ), bf16),
            pltpu.VMEM((8, D), f32),
            pltpu.VMEM((8, 128), jnp.int32),
            pltpu.VMEM((8, D), bf16),
            pltpu.VMEM((8, 128), f32),
            pltpu.VMEM((D, D), bf16),
            pltpu.VMEM((D, F), bf16),
            pltpu.VMEM((D, F), bf16),
            pltpu.VMEM((F, D), bf16),
            pltpu.SemaphoreType.DMA((4,)),
        ] + [pltpu.VMEM((S, TQ), f32)] * (2 * UB) + [pltpu.VMEM((8, TQ), f32)] * (2 * UB),
        compiler_params=pltpu.CompilerParams(
            dimension_semantics=("arbitrary",),
            vmem_limit_bytes=120 * 1024 * 1024),
    )(x, A_wqkv, A_wo, wr, B_w_gate, B_w_up, B_w_down)
    return out.reshape(1, S, D)
```

```python
import functools
import jax
import jax.numpy as jnp
import jax.experimental.pallas as pl
import jax.experimental.pallas.tpu as pltpu

S, D, H, DH, F = 2048, 512, 32, 16, 1792
G = 128 // DH
NG = H // G
LOG2E = 1.4426950408889634
bf16 = jnp.bfloat16
f32 = jnp.float32


def _rb(x):
    return x.astype(bf16).astype(f32)


def make_kernel(TQ, NC, UB, NXC, EARLY, TAPER):
    NQ = S // TQ
    NU = NQ * H
    KC = S // NC
    NQE = NQ
    XC = S // NXC

    def kernel(x_hbm, wqkv_hbm, wo_hbm, wr_ref, wg_hbm, wu_hbm, wd_hbm, o_hbm,
               x_ref, wqkv_ref, wqvt_ref, xn_ref, k_ref, qt_ref, vt_ref, ot_ref, r_ref, o_ref,
               wo_ref, wg_ref, wu_ref, wd_ref, sems, xsems, osems, *sm):
        s_refs = sm[:UB]
        m_refs = sm[UB:]
        late = [pltpu.make_async_copy(src, dst, sems.at[i]) for i, (src, dst) in enumerate(
            ((wo_hbm, wo_ref), (wg_hbm, wg_ref), (wu_hbm, wu_ref), (wd_hbm, wd_ref)))]
        w_cps = [pltpu.make_async_copy(wqkv_hbm.at[:, pl.ds(i * D, D)], wqkv_ref.at[:, pl.ds(i * D, D)], sems.at[4 + i])
                 for i in range(3)]
        x_cps = [pltpu.make_async_copy(x_hbm.at[pl.ds(c * XC, XC), :], x_ref.at[pl.ds(c * XC, XC), :], xsems.at[c])
                 for c in range(NXC)]
        o_cps = [pltpu.make_async_copy(o_ref.at[pl.ds(i * TQ, TQ), :], o_hbm.at[pl.ds(i * TQ, TQ), :], osems.at[i])
                 for i in range(NQ)]
        row = jax.lax.broadcasted_iota(jnp.int32, (128, TQ), 0) // DH

        def qmask(u):
            qq = u // H
            h = u % H
            g = h // G
            hh = h % G
            qg = qt_ref[qq, pl.ds(pl.multiple_of(g * 128, 128), 128), :]
            return g, jnp.where(row == hh, qg, jnp.zeros_like(qg))

        def qk(u, s_ref, m_ref):
            g, qm = qmask(u)
            s = jnp.dot(k_ref[g], qm, preferred_element_type=f32)
            s_ref[...] = s
            m_ref[...] = jnp.broadcast_to(jnp.max(s, axis=0, keepdims=True), (8, TQ))

        def layernorm(c):
            rs = slice(c * XC, (c + 1) * XC)
            xf = x_ref[rs, :].astype(f32)
            mean = jnp.mean(xf, axis=-1, keepdims=True)
            cen = xf - mean
            var = jnp.mean(cen * cen, axis=-1, keepdims=True)
            m_b = _rb(mean)
            v_b = _rb(var)
            d_b = _rb(xf - m_b)
            den = _rb(jnp.sqrt(_rb(v_b + 1e-5)))
            xn = (d_b / den).astype(bf16)
            xn_ref[rs, :] = xn
            return xn

        def project_k(c, xn):
            rs = slice(c * XC, (c + 1) * XC)
            k = jnp.dot(xn, wqkv_ref[:, D:2 * D], preferred_element_type=f32).astype(bf16)
            for g in range(NG):
                k_ref[g, rs, :] = k[:, g * 128:(g + 1) * 128]

        def project_qv(c, xn):
            rs = slice(c * XC, (c + 1) * XC)
            t = jax.lax.dot_general(wqvt_ref[...], xn, (((1,), (1,)), ((), ())), preferred_element_type=f32)
            qt = (_rb(t[0:D]) * (DH ** -0.5 * LOG2E)).astype(bf16)
            if XC >= TQ:
                for i in range(XC // TQ):
                    qt_ref[c * (XC // TQ) + i] = qt[:, i * TQ:(i + 1) * TQ]
            else:
                o = (c * XC) % TQ
                qt_ref[(c * XC) // TQ, :, o:o + XC] = qt
            vt_ref[:, rs] = t[D:2 * D].astype(bf16)
            r_ref[:, rs] = _rb(t[2 * D:2 * D + 8])

        def _prologue():
            x_cps[0].start()
            for i in (1, 0, 2):
                w_cps[i].start()
            if EARLY:
                for cp in x_cps[1:]:
                    cp.start()
            x_cps[0].wait()
            xn = layernorm(0)
            w_cps[1].wait()
            project_k(0, xn)
            w_cps[0].wait()
            w_cps[2].wait()
            if not EARLY:
                for cp in x_cps[1:]:
                    cp.start()
            wqvt_ref[0:D, :] = wqkv_ref[:, 0:D].T
            wqvt_ref[D:2 * D, :] = wqkv_ref[:, 2 * D:3 * D].T
            wqvt_ref[2 * D:2 * D + 16, :] = jnp.broadcast_to(wr_ref[...].reshape(1, D), (16, D))
            project_qv(0, xn)
            for cp in x_cps[1:]:
                cp.wait()
            for cp in late:
                cp.start()
            xn = layernorm(1)
            for c in range(1, NXC):
                xn_next = None
                if c + 1 < NXC:
                    xn_next = layernorm(c + 1)
                project_k(c, xn)
                project_qv(c, xn)
                xn = xn_next
            for t in range(UB):
                qk(t, s_refs[t], m_refs[t])

        _prologue()

        def block(pvs, qks):
            npv, nqk = len(pvs) * NC, len(qks) * NC
            qstate = {}
            qnext = 0
            for i, (u, b) in enumerate(pvs):
                sb = s_refs[b]
                mb_v = m_refs[b][0:1, :]
                h = u % H
                hrow = pl.multiple_of(h * DH, DH)
                oacc = None
                lacc = None
                for c in range(NC):
                    ks = slice(c * KC, (c + 1) * KC)
                    pf = jnp.exp2(sb[ks, :] - mb_v)
                    for r in reversed(range(KC // 8)):
                        lc = pf[8 * r:8 * r + 8, :]
                        lacc = lc if lacc is None else lacc + lc
                    p = pf.astype(bf16)
                    o = jnp.dot(vt_ref[pl.ds(hrow, DH), ks], p, preferred_element_type=f32)
                    oacc = o if oacc is None else oacc + o
                    slot = i * NC + c
                    while qnext < nqk and (qnext * npv) // nqk <= slot:
                        qi_, qc = divmod(qnext, NC)
                        u2, b2 = qks[qi_]
                        if qc == 0:
                            qstate[qi_] = qmask(u2) + (None,)
                        g, qm, macc = qstate[qi_]
                        qs = slice(qc * KC, (qc + 1) * KC)
                        sc = jnp.dot(k_ref[g, qs, :], qm, preferred_element_type=f32)
                        s_refs[b2][qs, :] = sc
                        mc = jnp.max(sc.reshape(KC // 8, 8, TQ), axis=0)
                        macc = mc if macc is None else jnp.maximum(macc, mc)
                        qstate[qi_] = (g, qm, macc)
                        if qc == NC - 1:
                            m_refs[b2][...] = jnp.broadcast_to(jnp.max(macc, axis=0, keepdims=True), (8, TQ))
                        qnext += 1
                o = oacc / jnp.sum(lacc, axis=0, keepdims=True)
                ot_ref[u // H, pl.ds(hrow, DH), :] = o.astype(bf16)

        def ffn():
            r = r_ref[...]
            rmax = jnp.max(r, axis=-1, keepdims=True)
            lane = jax.lax.broadcasted_iota(jnp.int32, (8, S), 1)
            idx = jnp.min(jnp.where(r == rmax, lane, S), axis=-1, keepdims=True)
            onehot = (lane == idx).astype(bf16)
            x_sel = jnp.dot(onehot, xn_ref[...], preferred_element_type=f32).astype(bf16)
            gg = _rb(jnp.dot(x_sel, wg_ref[...], preferred_element_type=f32))
            gg = _rb(gg * jax.nn.sigmoid(gg))
            uu = _rb(jnp.dot(x_sel, wu_ref[...], preferred_element_type=f32))
            gu = (gg * uu).astype(bf16)
            y = _rb(jnp.dot(gu, wd_ref[...], preferred_element_type=f32))
            y = _rb(y * _rb(jax.nn.sigmoid(rmax)))
            return idx[0:1, :], y[0:1, :]

        def epilogue(i, idx, y):
            rs = slice(i * TQ, (i + 1) * TQ)
            a = jax.lax.dot_general(ot_ref[i], wo_ref[...], (((0,), (0,)), ((), ())), preferred_element_type=f32)
            xt = x_ref[rs, :].astype(f32)
            xnt = xn_ref[rs, :].astype(f32)
            rows = jax.lax.broadcasted_iota(jnp.int32, (TQ, D), 0) + i * TQ
            upd = jnp.where(rows == idx, y, 0.0)
            o_ref[rs, :] = (_rb(xt + _rb(a)) + _rb(xnt + upd)).astype(o_ref.dtype)
            o_cps[i].start()

        assert sum(TAPER) == UB or not TAPER
        NB = (NU - UB - sum(TAPER)) // UB
        assert NB * UB + UB + sum(TAPER) == NU

        def body(j, carry):
            u = UB * j
            block([(u + t, t) for t in range(UB)], [(u + UB + t, t) for t in range(UB)])
            return carry

        jax.lax.fori_loop(0, NB, body, 0)

        u = NB * UB
        npend = UB
        for nq in TAPER:
            @pl.when(pl.program_id(0) == 0)
            def _():
                block([(u + t, (u + t) % UB) for t in range(npend)],
                      [(u + npend + t, (u + npend + t) % UB) for t in range(nq)])
            u += npend
            npend = nq

        for cp in late:
            cp.wait()
        block([(u + t, (u + t) % UB) for t in range(npend)], [])
        idx, y = ffn()
        for i in range(NQE):
            epilogue(i, idx, y)
        for cp in o_cps:
            cp.wait()

    return kernel, NQ


@jax.jit
def pallas_parallel_sum__softmax_full_mha__moe_arch_mod__prompt_kernel(
    A_x: jax.Array,
    A_wqkv: jax.Array,
    A_wo: jax.Array,
    B_x: jax.Array,
    B_w_r: jax.Array,
    B_w_gate: jax.Array,
    B_w_up: jax.Array,
    B_w_down: jax.Array,
):
    TQ, NC, UB, NXC, EARLY, TAPER = 256, 16, 8, 4, True, (4, 2, 1, 1)
    x = A_x.reshape(S, D)
    kernel, NQ = make_kernel(TQ, NC, UB, NXC, EARLY, TAPER)
    anyspec = pl.BlockSpec(memory_space=pl.ANY)
    out = pl.pallas_call(
        kernel,
        grid=(1,),
        in_specs=[anyspec, anyspec, anyspec, pl.BlockSpec((D,), lambda i: (0,)),
                  anyspec, anyspec, anyspec],
        out_specs=anyspec,
        out_shape=jax.ShapeDtypeStruct((S, D), bf16),
        scratch_shapes=[
            pltpu.VMEM((S, D), bf16),
            pltpu.VMEM((D, 3 * D), bf16),
            pltpu.VMEM((2 * D + 16, D), bf16),
            pltpu.VMEM((S, D), bf16),
            pltpu.VMEM((NG, S, 128), bf16),
            pltpu.VMEM((NQ, D, TQ), bf16),
            pltpu.VMEM((D, S), bf16),
            pltpu.VMEM((NQ, D, TQ), bf16),
            pltpu.VMEM((8, S), f32),
            pltpu.VMEM((S, D), bf16),
            pltpu.VMEM((D, D), bf16),
            pltpu.VMEM((D, F), bf16),
            pltpu.VMEM((D, F), bf16),
            pltpu.VMEM((F, D), bf16),
            pltpu.SemaphoreType.DMA((7,)),
            pltpu.SemaphoreType.DMA((NXC,)),
            pltpu.SemaphoreType.DMA((NQ,)),
        ] + [pltpu.VMEM((S, TQ), f32)] * UB + [pltpu.VMEM((8, TQ), f32)] * UB,
        compiler_params=pltpu.CompilerParams(
            dimension_semantics=("arbitrary",),
            vmem_limit_bytes=120 * 1024 * 1024),
    )(x, A_wqkv, A_wo, B_w_r, B_w_gate, B_w_up, B_w_down)
    return out.reshape(1, S, D)
```

```python
import jax
import jax.numpy as jnp
import jax.experimental.pallas as pl
import jax.experimental.pallas.tpu as pltpu

S, D, H, DH, F = 2048, 512, 32, 16, 1792
G = 128 // DH
NG = H // G
LOG2E = 1.4426950408889634
bf16 = jnp.bfloat16
f32 = jnp.float32

TQ = 256
NC = 16
UB = 8
NXC = 4
TAPER = (4, 2, 1, 1)

NQ = S // TQ
NU = NQ * H
KC = S // NC
XC = S // NXC
NB = (NU - UB - sum(TAPER)) // UB
assert UB % G == 0 and NB * UB + UB + sum(TAPER) == NU and XC % TQ == 0


def _rb(x):
    return x.astype(bf16).astype(f32)


def _kernel(x_hbm, wqkv_hbm, wo_hbm, wr_ref, wg_hbm, wu_hbm, wd_hbm, o_hbm,
            x_ref, wqkv_ref, wqvt_ref, xn_ref, k_ref, qt_ref, vt_ref, ot_ref, r_ref, o_ref,
            wo_ref, wg_ref, wu_ref, wd_ref, sems, xsems, osems, *sm):
    s_refs = sm[:UB]
    m_refs = sm[UB:]
    late = [pltpu.make_async_copy(src, dst, sems.at[i]) for i, (src, dst) in enumerate(
        ((wo_hbm, wo_ref), (wg_hbm, wg_ref), (wu_hbm, wu_ref), (wd_hbm, wd_ref)))]
    w_cps = [pltpu.make_async_copy(wqkv_hbm.at[:, pl.ds(i * D, D)], wqkv_ref.at[:, pl.ds(i * D, D)],
                                   sems.at[4 + i]) for i in range(3)]
    x_cps = [pltpu.make_async_copy(x_hbm.at[pl.ds(c * XC, XC), :], x_ref.at[pl.ds(c * XC, XC), :],
                                   xsems.at[c]) for c in range(NXC)]
    o_cps = [pltpu.make_async_copy(o_ref.at[pl.ds(i * TQ, TQ), :], o_hbm.at[pl.ds(i * TQ, TQ), :],
                                   osems.at[i]) for i in range(NQ)]

    def split(u):
        blk, t = u
        blk = blk + t // G
        t = t % G
        if isinstance(blk, int):
            return blk // NG, blk % NG, t
        return jnp.right_shift(blk, NG.bit_length() - 1), jnp.bitwise_and(blk, NG - 1), t

    def head_row(g, hh):
        r = g * 128 + hh * DH
        return r if isinstance(r, int) else pl.multiple_of(r, DH)

    def qmask(u):
        qq, g, hh = split(u)
        parts = [qt_ref[qq, pl.ds(head_row(g, hh), DH), :]]
        if hh > 0:
            parts.insert(0, jnp.zeros((hh * DH, TQ), bf16))
        if hh < G - 1:
            parts.append(jnp.zeros(((G - 1 - hh) * DH, TQ), bf16))
        return g, jnp.concatenate(parts, axis=0)

    def layernorm(c):
        rs = slice(c * XC, (c + 1) * XC)
        xf = x_ref[rs, :].astype(f32)
        mean = jnp.mean(xf, axis=-1, keepdims=True)
        cen = xf - mean
        var = jnp.mean(cen * cen, axis=-1, keepdims=True)
        d_b = _rb(xf - _rb(mean))
        den = _rb(jnp.sqrt(_rb(_rb(var) + 1e-5)))
        xn = (d_b / den).astype(bf16)
        xn_ref[rs, :] = xn
        return xn

    def project_k(c, xn):
        rs = slice(c * XC, (c + 1) * XC)
        k = jnp.dot(xn, wqkv_ref[:, D:2 * D], preferred_element_type=f32).astype(bf16)
        for g in range(NG):
            k_ref[g, rs, :] = k[:, g * 128:(g + 1) * 128]

    def project_qv(c, xn):
        rs = slice(c * XC, (c + 1) * XC)
        t = jax.lax.dot_general(wqvt_ref[...], xn, (((1,), (1,)), ((), ())), preferred_element_type=f32)
        qt = (_rb(t[0:D]) * (DH ** -0.5 * LOG2E)).astype(bf16)
        for i in range(XC // TQ):
            qt_ref[c * (XC // TQ) + i] = qt[:, i * TQ:(i + 1) * TQ]
        vt_ref[:, rs] = t[D:2 * D].astype(bf16)
        r_ref[:, rs] = _rb(t[2 * D:2 * D + 8])

    x_cps[0].start()
    w_cps[1].start()
    x_cps[1].start()
    w_cps[0].start()
    w_cps[2].start()
    for cp in x_cps[2:]:
        cp.start()
    x_cps[0].wait()
    xn0 = layernorm(0)
    w_cps[1].wait()
    x_cps[1].wait()
    xn1 = layernorm(1)
    project_k(0, xn0)
    project_k(1, xn1)
    w_cps[0].wait()
    w_cps[2].wait()
    for cp in x_cps[2:]:
        cp.wait()
    for cp in late:
        cp.start()
    wqvt_ref[0:D, :] = wqkv_ref[:, 0:D].T
    wqvt_ref[D:2 * D, :] = wqkv_ref[:, 2 * D:3 * D].T
    wqvt_ref[2 * D:2 * D + 16, :] = jnp.broadcast_to(wr_ref[...].reshape(1, D), (16, D))
    xn = layernorm(2)
    project_qv(0, xn0)
    project_qv(1, xn1)
    for c in range(2, NXC):
        xn_next = layernorm(c + 1) if c + 1 < NXC else None
        project_k(c, xn)
        project_qv(c, xn)
        xn = xn_next
    for t in range(UB):
        g, qm = qmask((0, t))
        s = jnp.dot(k_ref[g], qm, preferred_element_type=f32)
        s_refs[t][...] = s
        m_refs[t][...] = jnp.broadcast_to(jnp.max(s, axis=0, keepdims=True), (8, TQ))

    def block(pvs, qks):
        npv, nqk = len(pvs) * NC, len(qks) * NC
        qstate = {}
        qnext = 0
        for i, (u, b) in enumerate(pvs):
            sb = s_refs[b]
            mb_v = m_refs[b][0:1, :]
            uq, ug, uh = split(u)
            hrow = head_row(ug, uh)
            oacc = None
            lacc = None
            for c in range(NC):
                ks = slice(c * KC, (c + 1) * KC)
                pf = jnp.exp2(sb[ks, :] - mb_v)
                for r in reversed(range(KC // 8)):
                    lc = pf[8 * r:8 * r + 8, :]
                    lacc = lc if lacc is None else lacc + lc
                o = jnp.dot(vt_ref[pl.ds(hrow, DH), ks], pf.astype(bf16), preferred_element_type=f32)
                oacc = o if oacc is None else oacc + o
                slot = i * NC + c
                while qnext < nqk and (qnext * npv) // nqk <= slot:
                    qi, qc = divmod(qnext, NC)
                    u2, b2 = qks[qi]
                    if qc == 0:
                        qstate[qi] = qmask(u2) + (None,)
                    g, qm, macc = qstate[qi]
                    qs = slice(qc * KC, (qc + 1) * KC)
                    sc = jnp.dot(k_ref[g, qs, :], qm, preferred_element_type=f32)
                    s_refs[b2][qs, :] = sc
                    mc = jnp.max(sc.reshape(KC // 8, 8, TQ), axis=0)
                    macc = mc if macc is None else jnp.maximum(macc, mc)
                    qstate[qi] = (g, qm, macc)
                    if qc == NC - 1:
                        m_refs[b2][...] = jnp.broadcast_to(jnp.max(macc, axis=0, keepdims=True), (8, TQ))
                    qnext += 1
            o = oacc / jnp.sum(lacc, axis=0, keepdims=True)
            ot_ref[uq, pl.ds(hrow, DH), :] = o.astype(bf16)

    def body(j, carry):
        blk = j * (UB // G)
        block([((blk, t), t) for t in range(UB)], [((blk, UB + t), t) for t in range(UB)])
        return carry

    jax.lax.fori_loop(0, NB, body, 0)

    u = NB * UB
    npend = UB
    for nq in TAPER:
        block([((0, u + t), (u + t) % UB) for t in range(npend)],
              [((0, u + npend + t), (u + npend + t) % UB) for t in range(nq)])
        u += npend
        npend = nq
    for cp in late:
        cp.wait()
    block([((0, u + t), (u + t) % UB) for t in range(npend)], [])

    r = r_ref[...]
    rmax = jnp.max(r, axis=-1, keepdims=True)
    lane = jax.lax.broadcasted_iota(jnp.int32, (8, S), 1)
    idx = jnp.min(jnp.where(r == rmax, lane, S), axis=-1, keepdims=True)
    idx = jnp.minimum(idx, S - 1)
    blk16 = pl.multiple_of(jnp.bitwise_and(jnp.max(idx), -16), 16)
    lane16 = jax.lax.broadcasted_iota(jnp.int32, (8, 16), 1)
    onehot = (lane16 == jnp.bitwise_and(idx, 15)).astype(bf16)
    x_sel = jnp.dot(onehot, xn_ref[pl.ds(blk16, 16), :], preferred_element_type=f32).astype(bf16)
    gg = _rb(jnp.dot(x_sel, wg_ref[...], preferred_element_type=f32))
    gg = _rb(gg * jax.nn.sigmoid(gg))
    uu = _rb(jnp.dot(x_sel, wu_ref[...], preferred_element_type=f32))
    y = _rb(jnp.dot((gg * uu).astype(bf16), wd_ref[...], preferred_element_type=f32))
    y = _rb(y * _rb(jax.nn.sigmoid(rmax)))[0:1, :]
    idx = idx[0:1, :]

    for i in range(NQ):
        rs = slice(i * TQ, (i + 1) * TQ)
        a = jax.lax.dot_general(ot_ref[i], wo_ref[...], (((0,), (0,)), ((), ())), preferred_element_type=f32)
        xt = x_ref[rs, :].astype(f32)
        xnt = xn_ref[rs, :].astype(f32)
        rows = jax.lax.broadcasted_iota(jnp.int32, (TQ, D), 0) + i * TQ
        upd = jnp.where(rows == idx, y, 0.0)
        o_ref[rs, :] = (_rb(xt + _rb(a)) + _rb(xnt + upd)).astype(o_ref.dtype)
        o_cps[i].start()
    for cp in o_cps:
        cp.wait()


@jax.jit
def pallas_parallel_sum__softmax_full_mha__moe_arch_mod__prompt_kernel(
    A_x: jax.Array,
    A_wqkv: jax.Array,
    A_wo: jax.Array,
    B_x: jax.Array,
    B_w_r: jax.Array,
    B_w_gate: jax.Array,
    B_w_up: jax.Array,
    B_w_down: jax.Array,
):
    del B_x
    anyspec = pl.BlockSpec(memory_space=pl.ANY)
    out = pl.pallas_call(
        _kernel,
        grid=(1,),
        in_specs=[anyspec, anyspec, anyspec, pl.BlockSpec((D,), lambda i: (0,)),
                  anyspec, anyspec, anyspec],
        out_specs=anyspec,
        out_shape=jax.ShapeDtypeStruct((S, D), bf16),
        scratch_shapes=[
            pltpu.VMEM((S, D), bf16),
            pltpu.VMEM((D, 3 * D), bf16),
            pltpu.VMEM((2 * D + 16, D), bf16),
            pltpu.VMEM((S, D), bf16),
            pltpu.VMEM((NG, S, 128), bf16),
            pltpu.VMEM((NQ, D, TQ), bf16),
            pltpu.VMEM((D, S), bf16),
            pltpu.VMEM((NQ, D, TQ), bf16),
            pltpu.VMEM((8, S), f32),
            pltpu.VMEM((S, D), bf16),
            pltpu.VMEM((D, D), bf16),
            pltpu.VMEM((D, F), bf16),
            pltpu.VMEM((D, F), bf16),
            pltpu.VMEM((F, D), bf16),
            pltpu.SemaphoreType.DMA((7,)),
            pltpu.SemaphoreType.DMA((NXC,)),
            pltpu.SemaphoreType.DMA((NQ,)),
        ] + [pltpu.VMEM((S, TQ), f32)] * UB + [pltpu.VMEM((8, TQ), f32)] * UB,
        compiler_params=pltpu.CompilerParams(
            dimension_semantics=("arbitrary",),
            vmem_limit_bytes=100 * 1024 * 1024),
    )(A_x.reshape(S, D), A_wqkv, A_wo, B_w_r, B_w_gate, B_w_up, B_w_down)
    return out.reshape(1, S, D)
```
